```python
import os as _os
_os.environ.setdefault('JAX_PLATFORMS', 'cpu')
import jax
import jax.numpy as jnp

def _softmax(x, axis=-1):
    return jax.nn.softmax(x, axis=axis)

def _gelu(x):
    return jax.nn.gelu(x, approximate=True)

def _silu(x):
    return jax.nn.silu(x)

def _sigmoid(x):
    return jax.nn.sigmoid(x)

def _layernorm(x, axis=-1, eps=1e-05):
    m = jnp.mean(x, axis=axis, keepdims=True)
    v = jnp.var(x, axis=axis, keepdims=True)
    return (x - m) / jnp.sqrt(v + eps)

def _scatter_add(tgt, idx, src, axis=0):
    return tgt.at[idx].add(src)

def _segment_sum(src, seg, n):
    return jax.ops.segment_sum(src, seg, n)

class _Rng:

    def __init__(self, key):
        self._k = key

    def _next(self):
        self._k, sub = jax.random.split(self._k)
        return sub

    def normal(self, shape):
        return jax.random.normal(self._next(), shape, dtype=jnp.bfloat16)

    def randint(self, lo, hi, shape):
        return jax.random.randint(self._next(), shape, lo, hi, dtype=jnp.int32)

    def uniform(self, shape, lo=0.0, hi=1.0):
        return jax.random.uniform(self._next(), shape, jnp.bfloat16, lo, hi)

    def permutation(self, n):
        return jax.random.permutation(self._next(), n)
kernel_name = 'sequential_preLN__memory_aug_recurrent_mem_tr__swiglu_ffn__prompt'

def setup_inputs():
    _rng = _Rng(jax.random.key(int.from_bytes(__import__("os").urandom(4), "little")))
    _w = lambda a: (lambda t: t.astype(jnp.bfloat16) if jnp.issubdtype(t.dtype, jnp.floating) else t)(jnp.asarray(a))

    def _A_setup():
        B, S, Dm = (1, 2048, 640)
        H, Dh = (32, 192)
        M, seg = (8, 32)
        seg = min(seg, S)
        S = S // seg * seg
        return {'x': _w((lambda *s: _rng.normal(s) * 0.05)(B, S, Dm)), 'mem0': _w((lambda *s: _rng.normal(s) * 0.1)(B, M, Dm)), 'Wq': _w((lambda *s: _rng.normal(s) * 1.6)(Dm, H, Dh) * Dm ** (-0.5)), 'Wk': _w((lambda *s: _rng.normal(s) * 1.6)(Dm, H, Dh) * Dm ** (-0.5)), 'Wv': _w((lambda *s: _rng.normal(s) * 0.1)(Dm, H, Dh) * Dm ** (-0.5)), 'Wo': _w((lambda *s: _rng.normal(s) * 0.1)(H, Dh, Dm) * (H * Dh) ** (-0.5)), 'seg_len': seg}
    _A_in = _A_setup()

    def _B_setup():
        B, S, D, F = (1, 2048, 640, 1536)
        return {'x': _w((lambda *s: _rng.normal(s) * 0.05)(B, S, D)), 'w_gate': _w((lambda *s: _rng.normal(s) * 0.05)(D, F)), 'w_up': _w((lambda *s: _rng.normal(s) * 0.05)(D, F)), 'w_down': _w((lambda *s: _rng.normal(s) * 0.05)(F, D))}
    _B_in = _B_setup()
    return {'A_x': _A_in['x'], 'A_mem0': _A_in['mem0'], 'A_Wq': _A_in['Wq'], 'A_Wk': _A_in['Wk'], 'A_Wv': _A_in['Wv'], 'A_Wo': _A_in['Wo'], 'A_seg_len': _A_in['seg_len'], 'B_x': _B_in['x'], 'B_w_gate': _B_in['w_gate'], 'B_w_up': _B_in['w_up'], 'B_w_down': _B_in['w_down']}

def reference(A_x, A_mem0, A_Wq, A_Wk, A_Wv, A_Wo, A_seg_len, B_x, B_w_gate, B_w_up, B_w_down):

    def _A_ref(x, mem0, Wq, Wk, Wv, Wo, seg_len):
        B, S, Dm = x.shape
        H, Dh = (Wq.shape[1], Wq.shape[2])
        M = mem0.shape[1]
        scale = Dh ** (-0.5)
        n_seg = S // seg_len
        L = M + seg_len
        idx = jnp.arange(L)
        mask = (idx[:, None] < M) | (idx[:, None] >= idx[None, :])
        mem = mem0
        outs = []
        for s in range(n_seg):
            xs = x[:, s * seg_len:(s + 1) * seg_len, :].copy()
            h = jnp.concatenate([mem, xs], axis=1)
            q = jnp.einsum('btd,dhe->bhte', h, Wq)
            k = jnp.einsum('btd,dhe->bhte', h, Wk)
            v = jnp.einsum('btd,dhe->bhte', h, Wv)
            scores = jnp.einsum('bhqe,bhke->bhqk', q, k) * scale
            scores = jnp.where(mask[None, None], scores, -1000000000.0)
            p = _softmax(scores, axis=-1)
            o = jnp.einsum('bhqk,bhke->bhqe', p, v)
            o = jnp.einsum('bhte,hed->btd', o, Wo)
            mem = o[:, :M, :].copy()
            outs.append(o[:, M:, :])
        return jnp.concatenate(outs, axis=1)

    def _B_ref(x, w_gate, w_up, w_down):
        g = _silu(x @ w_gate)
        u = x @ w_up
        return g * u @ w_down
    x = A_x
    h = x + _A_ref(_layernorm(x, axis=-1), A_mem0, A_Wq, A_Wk, A_Wv, A_Wo, A_seg_len)
    h2 = h + _B_ref(_layernorm(h, axis=-1), B_w_gate, B_w_up, B_w_down)
    return h2
```

```python
import functools
import numpy as np
import jax
import jax.numpy as jnp
from jax import lax
import jax.experimental.pallas as pl
import jax.experimental.pallas.tpu as pltpu

F32 = jnp.float32
BF16 = jnp.bfloat16


def _mm(a, b):
    return lax.dot_general(a, b, (((1,), (0,)), ((), ())), preferred_element_type=F32)


def _mm_nt(a, b):
    return lax.dot_general(a, b, (((1,), (1,)), ((), ())), preferred_element_type=F32)


def _ln(x):
    m = jnp.mean(x, axis=-1, keepdims=True)
    d = x - m
    v = jnp.mean(d * d, axis=-1, keepdims=True)
    return d * lax.rsqrt(v + 1e-5)


def _kernel(x_hbm, mem0_ref, wq_hbm, wk_hbm, wv_hbm, wo_hbm, wg_hbm, wu_hbm, wd_hbm,
            out_hbm,
            x_v, xn_v, h_v, out_v, stg, wqkv, wo, wg, wu, wd, sem_w, sem_m,
            *, S, Dm, H, Dh, M, seg, F):
    NP = H // 2
    PW = 2 * Dh
    L = M + seg
    n_seg = S // seg
    scale = Dh ** (-0.5)

    cp_x = pltpu.make_async_copy(x_hbm, x_v, sem_m.at[0])
    cp_x.start()

    def wcopy(i, j):
        src = (wq_hbm, wk_hbm, wv_hbm)[i]
        return pltpu.make_async_copy(src.at[pl.ds(j * PW, PW), :], stg.at[i, j], sem_w.at[i * NP + j])

    def ocopy(j):
        return pltpu.make_async_copy(wo_hbm.at[pl.ds(j * PW, PW), :], wo.at[j], sem_w.at[3 * NP + j])

    for j in range(NP):
        for i in range(3):
            wcopy(i, j).start()
    for j in range(NP):
        ocopy(j).start()
    cp_g = pltpu.make_async_copy(wg_hbm, wg, sem_m.at[1])
    cp_u = pltpu.make_async_copy(wu_hbm, wu, sem_m.at[2])
    cp_d = pltpu.make_async_copy(wd_hbm, wd, sem_m.at[3])
    cp_g.start(); cp_u.start(); cp_d.start()

    cp_x.wait()
    RB = 64

    def ln_body(i, c):
        r = pl.multiple_of(i * RB, RB)
        xn_v[pl.ds(r, RB), :] = _ln(x_v[pl.ds(r, RB), :].astype(F32))
        return c
    lax.fori_loop(0, S // RB, ln_body, 0)
    h_v[...] = jnp.zeros(h_v.shape, F32)

    def tr_body(j, c):
        for i in range(3):
            pltpu.make_async_copy(stg.at[i, j], stg.at[i, j], sem_w.at[i * NP + j]).wait()
            for t in range(PW // 128):
                blk = stg[i, j, t * 128:(t + 1) * 128, :]
                wqkv[j, :, i * PW + t * 128:i * PW + (t + 1) * 128] = blk.astype(F32).T.astype(BF16)
        return c
    lax.fori_loop(0, NP, tr_body, 0)
    for j in range(NP):
        ocopy(j).wait()
    cp_g.wait(); cp_u.wait(); cp_d.wait()

    row = lax.broadcasted_iota(jnp.int32, (2 * L, 2 * L), 0)
    col = lax.broadcasted_iota(jnp.int32, (2 * L, 2 * L), 1)
    same = (row >= L) == (col >= L)
    r_in = jnp.where(row >= L, row - L, row)
    c_in = jnp.where(col >= L, col - L, col)
    valid = same & ((r_in < M) | (r_in >= c_in))
    fill = jnp.where(same, jnp.float32(-1e9), jnp.float32(-jnp.inf))
    lo = lax.broadcasted_iota(jnp.int32, (L, 128), 1) < (Dh - 128)

    NF = 3
    FC = F // NF

    def ffn_gu(hn, c):
        g = _mm(hn, wg[:, c * FC:(c + 1) * FC])
        u = _mm(hn, wu[:, c * FC:(c + 1) * FC])
        return g * (1.0 / (1.0 + jnp.exp(-g))) * u

    def ffn_down(hprev, acts):
        y = hprev
        for c in range(NF):
            y = y + _mm(acts[c], wd[c * FC:(c + 1) * FC, :])
        return y

    def step(s, mem):
        r = pl.multiple_of(s * seg, seg)
        rp = pl.multiple_of(jnp.maximum(s - 1, 0) * seg, seg)
        hin = jnp.concatenate([mem, xn_v[pl.ds(r, seg), :]], axis=0)
        hprev = h_v[...]
        hn = _ln(hprev)
        st = {}

        def A(j):
            st['qkv', j] = _mm(hin, wqkv[j])

        def QK(j):
            y = st.pop(('qkv', j))
            t = [y[:, i * 128:(i + 1) * 128] for i in range(9)]
            qm = jnp.concatenate([t[0], t[2]], axis=0)
            km = jnp.concatenate([t[3], t[5]], axis=0).astype(BF16)
            kt = jnp.concatenate([jnp.where(lo, t[4], 0.0), jnp.where(lo, 0.0, t[4])], axis=0).astype(BF16)
            st['vm', j] = jnp.concatenate([t[6], t[8]], axis=0).astype(BF16)
            st['vt', j] = jnp.concatenate([jnp.where(lo, t[7], 0.0), jnp.where(lo, 0.0, t[7])], axis=0).astype(BF16)
            sm = _mm_nt(qm, km)
            stl = _mm_nt(t[1], kt)
            sc = (sm + jnp.concatenate([stl, stl], axis=0)) * scale
            sc = jnp.where(valid, sc, fill)
            mx = jnp.max(sc, axis=-1, keepdims=True)
            e = jnp.exp(sc - mx)
            p = e / jnp.sum(e, axis=-1, keepdims=True)
            st['p', j] = p

        def PV(j):
            p = st.pop(('p', j))
            om = _mm(p, st.pop(('vm', j)))
            ot = _mm(p[:L] + p[L:], st.pop(('vt', j)))
            st['o', j] = jnp.concatenate([om[:L], ot, om[L:]], axis=1)

        def C(j):
            y = _mm(st.pop(('o', j)), wo[j])
            st['acc'] = y if j == 0 else st['acc'] + y

        acts = []
        for t in range(NP + 3):
            if t < NP:
                A(t)
            else:
                acts.append(ffn_gu(hn, t - NP))
            if 0 <= t - 3 < NP:
                C(t - 3)
            if 0 <= t - 2 < NP:
                PV(t - 2)
            if 0 <= t - 1 < NP:
                QK(t - 1)
        out_v[pl.ds(rp, seg), :] = ffn_down(hprev, acts).astype(BF16)
        acc = st['acc']
        h_v[...] = x_v[pl.ds(r, seg), :].astype(F32) + acc[M:]
        return acc[:M]

    lax.fori_loop(0, n_seg, step, mem0_ref[...].astype(F32))
    hprev = h_v[...]
    hn = _ln(hprev)
    acts = [ffn_gu(hn, c) for c in range(NF)]
    out_v[S - seg:, :] = ffn_down(hprev, acts).astype(BF16)
    cp_o = pltpu.make_async_copy(out_v, out_hbm, sem_m.at[0])
    cp_o.start()
    cp_o.wait()


@functools.partial(jax.jit, static_argnames=("A_seg_len",))
def pallas_sequential_preLN__memory_aug_recurrent_mem_tr__swiglu_ffn__prompt_kernel(A_x, A_mem0, A_Wq, A_Wk, A_Wv, A_Wo, A_seg_len, B_x, B_w_gate, B_w_up, B_w_down):
    B, S, Dm = A_x.shape
    _, H, Dh = A_Wq.shape
    M = A_mem0.shape[1]
    F = B_w_gate.shape[1]
    seg = A_seg_len
    NP, PW = H // 2, 2 * Dh
    wt = lambda w: jnp.transpose(w, (1, 2, 0)).reshape(H * Dh, Dm)
    anyspec = pl.BlockSpec(memory_space=pl.ANY)
    out = pl.pallas_call(
        functools.partial(_kernel, S=S, Dm=Dm, H=H, Dh=Dh, M=M, seg=seg, F=F),
        out_shape=jax.ShapeDtypeStruct((S, Dm), A_x.dtype),
        in_specs=[anyspec, pl.BlockSpec(memory_space=pltpu.VMEM)] + [anyspec] * 7,
        out_specs=anyspec,
        scratch_shapes=[
            pltpu.VMEM((S, Dm), BF16),
            pltpu.VMEM((S, Dm), F32),
            pltpu.VMEM((seg, Dm), F32),
            pltpu.VMEM((S, Dm), BF16),
            pltpu.VMEM((3, NP, PW, Dm), BF16),
            pltpu.VMEM((NP, Dm, 3 * PW), BF16),
            pltpu.VMEM((NP, PW, Dm), BF16),
            pltpu.VMEM((Dm, F), BF16),
            pltpu.VMEM((Dm, F), BF16),
            pltpu.VMEM((F, Dm), BF16),
            pltpu.SemaphoreType.DMA((4 * NP,)),
            pltpu.SemaphoreType.DMA((4,)),
        ],
        compiler_params=pltpu.CompilerParams(vmem_limit_bytes=110 << 20),
    )(A_x.reshape(S, Dm), A_mem0.reshape(M, Dm), wt(A_Wq), wt(A_Wk), wt(A_Wv),
      A_Wo.reshape(H * Dh, Dm), B_w_gate, B_w_up, B_w_down)
    return out.reshape(B, S, Dm)
```

```python
import functools
import itertools
import numpy as np
import jax
import jax.numpy as jnp
from jax import lax
import jax.experimental.pallas as pl
import jax.experimental.pallas.tpu as pltpu

F32 = jnp.float32
BF16 = jnp.bfloat16
U32 = jnp.uint32
RING = 4
PERMS = [a + ''.join(p) for a in 'A' for p in itertools.permutations('CPQ')]
ORDER = 1
LAG = 134
NF = 4
UNROLL = 4


def _mm(a, b):
    return lax.dot_general(a, b, (((1,), (0,)), ((), ())), preferred_element_type=F32)


def _mm_nt(a, b):
    return lax.dot_general(a, b, (((1,), (1,)), ((), ())), preferred_element_type=F32)


def _ln(x):
    m = jnp.mean(x, axis=-1, keepdims=True)
    d = x - m
    v = jnp.mean(d * d, axis=-1, keepdims=True)
    return d * lax.rsqrt(v + 1e-5)


def _kernel(x_hbm, mem0_ref, wq_hbm, wk_hbm, wv_hbm, wo_hbm, wg_hbm, wu_hbm, wd_hbm,
            out_hbm,
            x_v, xq_v, xp_v, pre, h_v, out_v, stg, wqkv, wo, wg, wu, wd, sem_w, sem_o, sem_f, sem_m,
            *, S, Dm, H, Dh, M, seg, F):
    NP = H // 2
    PW = 2 * Dh
    L = M + seg
    n_seg = S // seg
    scale = Dh ** (-0.5)
    PR = M
    GR = 48
    NG = -(-Dm // GR)

    def wcopies(j):
        slot = j % RING
        return [pltpu.make_async_copy(src.at[pl.ds(j * PW, PW), :], stg.at[slot, i], sem_w.at[slot * 3 + i])
                for i, src in enumerate((wq_hbm, wk_hbm, wv_hbm))]

    cp_p = pltpu.make_async_copy(x_hbm.at[:, pl.ds(0, PR), :], xq_v, sem_m.at[2])
    cp_x = pltpu.make_async_copy(x_hbm, x_v, sem_m.at[0])
    cp_p.start()
    wcopies(0)[0].start()
    h_v[...] = jnp.zeros(h_v.shape, F32)
    cp_p.wait()
    for c in wcopies(0)[1:]:
        c.start()
    for i in range(n_seg * PR // 128):
        xs = jnp.concatenate([xq_v[i * (128 // PR) + t].astype(F32) for t in range(128 // PR)], axis=0)
        xp_v[i * 128:(i + 1) * 128, :] = _ln(xs).astype(BF16)

    def transpose_pair(j):
        slot = j % RING
        for i in range(3):
            for t in range(PW // 128):
                blk = stg[slot, i, t * 128:(t + 1) * 128, :]
                wqkv[j, :, i * PW + t * 128:i * PW + (t + 1) * 128] = pltpu.bitcast(
                    blk.astype(F32).T.astype(BF16), U32)

    def project_pre(j):
        w = pltpu.bitcast(wqkv[j], BF16)
        for c in range(n_seg * PR // 128):
            pre[j, c * 128:(c + 1) * 128, :] = _mm(xp_v[c * 128:(c + 1) * 128, :], w)

    OB = H * Dh // NP
    DB = F // NP

    GB = Dm // NP

    def side_copies(j):
        return [pltpu.make_async_copy(wo_hbm.at[pl.ds(j * OB, OB), :], wo.at[j], sem_o.at[0]),
                pltpu.make_async_copy(wd_hbm.at[pl.ds(j * DB, DB), :], wd.at[pl.ds(j * DB, DB), :], sem_f.at[0]),
                pltpu.make_async_copy(wg_hbm.at[pl.ds(j * GB, GB), :], wg.at[pl.ds(j * GB, GB), :], sem_f.at[1]),
                pltpu.make_async_copy(wu_hbm.at[pl.ds(j * GB, GB), :], wu.at[pl.ds(j * GB, GB), :], sem_f.at[2])]

    for c in wcopies(0):
        c.wait()
    for j in range(1, RING):
        for c in wcopies(j):
            c.start()
    cp_x.start()
    transpose_pair(0)

    def pro_body(j, c, refill):
        for cp in wcopies(j + 1):
            cp.wait()
        if refill:
            for cp in wcopies(j + RING):
                cp.start()
        for cp in side_copies(j):
            cp.start()
        transpose_pair(j + 1)
        project_pre(j)
        return c
    lax.fori_loop(0, NP - RING, functools.partial(pro_body, refill=True), 0)
    lax.fori_loop(NP - RING, NP - 1, functools.partial(pro_body, refill=False), 0)
    for cp in side_copies(NP - 1):
        cp.start()
    project_pre(NP - 1)
    pltpu.make_async_copy(wo, wo, sem_o.at[0]).wait()
    pltpu.make_async_copy(wd, wd, sem_f.at[0]).wait()
    cp_x.wait()
    pltpu.make_async_copy(wg, wg, sem_f.at[1]).wait()
    pltpu.make_async_copy(wu, wu, sem_f.at[2]).wait()

    row = lax.broadcasted_iota(jnp.int32, (2 * L, 2 * L), 0)
    col = lax.broadcasted_iota(jnp.int32, (2 * L, 2 * L), 1)
    same = (row >= L) == (col >= L)
    r_in = jnp.where(row >= L, row - L, row)
    c_in = jnp.where(col >= L, col - L, col)
    valid = same & ((r_in < M) | (r_in >= c_in))
    fill = jnp.where(same, jnp.float32(-1e9), jnp.float32(-jnp.inf))
    lo = lax.broadcasted_iota(jnp.int32, (L, 128), 1) < (Dh - 128)

    FC = F // NF

    def ffn_gu(hn, c):
        g = _mm(hn, wg[:, c * FC:(c + 1) * FC])
        u = _mm(hn, wu[:, c * FC:(c + 1) * FC])
        return (g * (1.0 / (1.0 + jnp.exp(-g))) * u).astype(BF16)

    def ffn_down(hprev, acts):
        y = hprev
        for c in range(NF):
            y = y + _mm(acts[c], wd[c * FC:(c + 1) * FC, :])
        return y

    OR = UNROLL * seg

    def ocopy(i):
        r = pl.ds(pl.multiple_of(i * OR, OR), OR)
        return pltpu.make_async_copy(out_v.at[r, :], out_hbm.at[r, :], sem_m.at[1])

    def lhs(mem, s):
        return jnp.concatenate([mem, _ln(x_v[s, PR:, :].astype(F32))], axis=0).astype(BF16)

    def step(s, hin):
        rp = pl.multiple_of(jnp.maximum(s - 1, 0) * seg, seg)
        rq = pl.multiple_of(s * PR, PR)
        hprev = h_v[...]
        hn = _ln(hprev).astype(BF16)
        st = {}

        def A(j):
            y = _mm(hin, pltpu.bitcast(wqkv[j], BF16))
            st['qkv', j] = jnp.concatenate([y[:M], pre[j, pl.ds(rq, PR), :], y[M:]], axis=0)

        def QK(j):
            y = st.pop(('qkv', j))
            t = [y[:, i * 128:(i + 1) * 128] for i in range(9)]
            qm = jnp.concatenate([t[0], t[2]], axis=0)
            km = jnp.concatenate([t[3], t[5]], axis=0).astype(BF16)
            kt = jnp.concatenate([jnp.where(lo, t[4], 0.0), jnp.where(lo, 0.0, t[4])], axis=0).astype(BF16)
            st['vm', j] = jnp.concatenate([t[6], t[8]], axis=0).astype(BF16)
            st['vt', j] = jnp.concatenate([jnp.where(lo, t[7], 0.0), jnp.where(lo, 0.0, t[7])], axis=0).astype(BF16)
            sm = _mm_nt(qm, km)
            stl = _mm_nt(t[1], kt)
            sc = (sm + jnp.concatenate([stl, stl], axis=0)) * scale
            sc = jnp.where(valid, sc, fill)
            mx = jnp.max(sc, axis=-1, keepdims=True)
            e = jnp.exp(sc - mx)
            p = e / jnp.sum(e, axis=-1, keepdims=True)
            st['p', j] = p

        def PV(j):
            p = st.pop(('p', j))
            om = _mm(p, st.pop(('vm', j)))
            ot = _mm(p[:L] + p[L:], st.pop(('vt', j)))
            st['o', j] = jnp.concatenate([om[:L], ot, om[L:]], axis=1)

        def C(j):
            y = _mm(st.pop(('o', j)), wo[j])
            st['acc'] = y if j == 0 else st['acc'] + y

        acts = []
        lq, lp, lc = LAG // 100, LAG // 10 % 10, LAG % 10
        for t in range(NP + lc):
            for op in PERMS[ORDER]:
                if op == 'A':
                    if t < NP:
                        A(t)
                    elif t - NP < NF:
                        acts.append(ffn_gu(hn, t - NP))
                elif op == 'C' and 0 <= t - lc < NP:
                    C(t - lc)
                elif op == 'P' and 0 <= t - lp < NP:
                    PV(t - lp)
                elif op == 'Q' and 0 <= t - lq < NP:
                    QK(t - lq)
        while len(acts) < NF:
            acts.append(ffn_gu(hn, len(acts)))
        out_v[pl.ds(rp, seg), :] = ffn_down(hprev, acts).astype(BF16)
        acc = st['acc']
        h_v[...] = x_v[s].astype(F32) + acc[M:]
        return lhs(acc[:M], jnp.minimum(s + 1, n_seg - 1))

    def steps(i, hin):
        @pl.when(i >= 2)
        def _():
            ocopy(i - 2).start()
        for u in range(UNROLL):
            hin = step(i * UNROLL + u, hin)
        return hin

    n_it = n_seg // UNROLL
    lax.fori_loop(0, n_it, steps, lhs(mem0_ref[...].astype(F32), 0))
    ocopy(n_it - 2).start()
    hprev = h_v[...]
    hn = _ln(hprev).astype(BF16)
    acts = [ffn_gu(hn, c) for c in range(NF)]
    out_v[S - seg:, :] = ffn_down(hprev, acts).astype(BF16)
    ocopy(n_it - 1).start()
    pltpu.make_async_copy(out_v, out_hbm, sem_m.at[1]).wait()


@functools.partial(jax.jit, static_argnames=("A_seg_len",))
def pallas_sequential_preLN__memory_aug_recurrent_mem_tr__swiglu_ffn__prompt_kernel(A_x, A_mem0, A_Wq, A_Wk, A_Wv, A_Wo, A_seg_len, B_x, B_w_gate, B_w_up, B_w_down):
    B, S, Dm = A_x.shape
    _, H, Dh = A_Wq.shape
    M = A_mem0.shape[1]
    F = B_w_gate.shape[1]
    seg = A_seg_len
    NP, PW = H // 2, 2 * Dh
    n_seg = S // seg
    wt = lambda w: jnp.transpose(w, (1, 2, 0)).reshape(H * Dh, Dm)
    anyspec = pl.BlockSpec(memory_space=pl.ANY)
    out = pl.pallas_call(
        functools.partial(_kernel, S=S, Dm=Dm, H=H, Dh=Dh, M=M, seg=seg, F=F),
        out_shape=jax.ShapeDtypeStruct((S, Dm), A_x.dtype),
        in_specs=[anyspec, pl.BlockSpec(memory_space=pltpu.VMEM)] + [anyspec] * 7,
        out_specs=anyspec,
        scratch_shapes=[
            pltpu.VMEM((n_seg, seg, Dm), BF16),
            pltpu.VMEM((n_seg, M, Dm), BF16),
            pltpu.VMEM((n_seg * M, Dm), BF16),
            pltpu.VMEM((NP, n_seg * M, 3 * PW), F32),
            pltpu.VMEM((seg, Dm), F32),
            pltpu.VMEM((S, Dm), BF16),
            pltpu.VMEM((RING, 3, PW, Dm), BF16),
            pltpu.VMEM((NP, Dm // 2, 3 * PW), U32),
            pltpu.VMEM((NP, PW, Dm), BF16),
            pltpu.VMEM((Dm, F), BF16),
            pltpu.VMEM((Dm, F), BF16),
            pltpu.VMEM((F, Dm), BF16),
            pltpu.SemaphoreType.DMA((RING * 3,)),
            pltpu.SemaphoreType.DMA((1,)),
            pltpu.SemaphoreType.DMA((3,)),
            pltpu.SemaphoreType.DMA((3,)),
        ],
        compiler_params=pltpu.CompilerParams(vmem_limit_bytes=110 << 20, disable_bounds_checks=True,
            flags={'XLA_TPU_EVENLY_DISTRIBUTE_CRITICAL_NODES': True}),
    )(A_x.reshape(n_seg, seg, Dm), A_mem0.reshape(M, Dm), wt(A_Wq), wt(A_Wk), wt(A_Wv),
      A_Wo.reshape(H * Dh, Dm), B_w_gate, B_w_up, B_w_down)
    return out.reshape(B, S, Dm)
```

```python
import functools
import itertools
import numpy as np
import jax
import jax.numpy as jnp
from jax import lax
import jax.experimental.pallas as pl
import jax.experimental.pallas.tpu as pltpu

F32 = jnp.float32
BF16 = jnp.bfloat16
U32 = jnp.uint32
RING = 4
PERMS = [a + ''.join(p) for a in 'A' for p in itertools.permutations('CPQ')]
ORDER = 1
LAG = 134
NF = 4
UNROLL = 4


def _mm(a, b):
    return lax.dot_general(a, b, (((1,), (0,)), ((), ())), preferred_element_type=F32)


def _mm_nt(a, b):
    return lax.dot_general(a, b, (((1,), (1,)), ((), ())), preferred_element_type=F32)


def _ln(x):
    m = jnp.mean(x, axis=-1, keepdims=True)
    d = x - m
    v = jnp.mean(d * d, axis=-1, keepdims=True)
    return d * lax.rsqrt(v + 1e-5)


def _kernel(x_hbm, mem0_ref, wq_hbm, wk_hbm, wv_hbm, wo_hbm, wg_hbm, wu_hbm, wd_hbm,
            out_hbm,
            x_v, xq_v, xp_v, pre, h_v, out_v, stg, wqkv, wo, wg, wu, wd, sem_w, sem_o, sem_f, sem_m,
            *, S, Dm, H, Dh, M, seg, F):
    NP = H // 2
    PW = 2 * Dh
    L = M + seg
    n_seg = S // seg
    scale = Dh ** (-0.5)
    PR = M
    GR = 48
    NG = -(-Dm // GR)

    def wcopies(j):
        slot = j % RING
        return [pltpu.make_async_copy(src.at[pl.ds(j * PW, PW), :], stg.at[slot, i], sem_w.at[slot * 3 + i])
                for i, src in enumerate((wq_hbm, wk_hbm, wv_hbm))]

    cp_p = pltpu.make_async_copy(x_hbm.at[:, pl.ds(0, PR), :], xq_v, sem_m.at[2])
    cp_x = pltpu.make_async_copy(x_hbm, x_v, sem_m.at[0])
    cp_p.start()
    wcopies(0)[0].start()
    h_v[...] = jnp.zeros(h_v.shape, F32)
    cp_p.wait()
    for c in wcopies(0)[1:]:
        c.start()
    for i in range(n_seg * PR // 128):
        xs = jnp.concatenate([xq_v[i * (128 // PR) + t].astype(F32) for t in range(128 // PR)], axis=0)
        xp_v[i * 128:(i + 1) * 128, :] = _ln(xs).astype(BF16)

    def transpose_w(j, i):
        slot = j % RING
        for t in range(PW // 128):
            blk = stg[slot, i, t * 128:(t + 1) * 128, :]
            wqkv[j, :, i * PW + t * 128:i * PW + (t + 1) * 128] = pltpu.bitcast(
                blk.astype(F32).T.astype(BF16), U32)

    def transpose_pair(j):
        for i in range(3):
            transpose_w(j, i)

    def project_pre(j, c0=0, c1=3 * PW):
        w = pltpu.bitcast(wqkv[j, :, c0:c1], BF16)
        for c in range(n_seg * PR // 128):
            pre[j, c * 128:(c + 1) * 128, c0:c1] = _mm(xp_v[c * 128:(c + 1) * 128, :], w)

    OB = H * Dh // NP
    DB = F // NP

    GB = Dm // NP

    def side_copies(j):
        return [pltpu.make_async_copy(wo_hbm.at[pl.ds(j * OB, OB), :], wo.at[j], sem_o.at[0]),
                pltpu.make_async_copy(wd_hbm.at[pl.ds(j * DB, DB), :], wd.at[pl.ds(j * DB, DB), :], sem_f.at[0]),
                pltpu.make_async_copy(wg_hbm.at[pl.ds(j * GB, GB), :], wg.at[pl.ds(j * GB, GB), :], sem_f.at[1]),
                pltpu.make_async_copy(wu_hbm.at[pl.ds(j * GB, GB), :], wu.at[pl.ds(j * GB, GB), :], sem_f.at[2])]

    w0 = wcopies(0)
    w0[0].wait()
    for c in wcopies(1):
        c.start()
    transpose_w(0, 0)
    project_pre(0, 0, PW)
    w0[1].wait()
    w0[2].wait()
    for j in range(2, RING):
        for c in wcopies(j):
            c.start()
    transpose_w(0, 1)
    transpose_w(0, 2)
    project_pre(0, PW, 2 * PW)
    for c in wcopies(1):
        c.wait()
    for c in wcopies(RING) + side_copies(0) + [cp_x]:
        c.start()
    transpose_pair(1)
    project_pre(0, 2 * PW, 3 * PW)

    def pro_body(j, c, refill):
        for cp in wcopies(j + 1):
            cp.wait()
        if refill:
            for cp in wcopies(j + RING):
                cp.start()
        for cp in side_copies(j):
            cp.start()
        transpose_pair(j + 1)
        project_pre(j)
        return c
    lax.fori_loop(1, NP - RING, functools.partial(pro_body, refill=True), 0)
    lax.fori_loop(NP - RING, NP - 1, functools.partial(pro_body, refill=False), 0)
    for cp in side_copies(NP - 1):
        cp.start()
    project_pre(NP - 1)
    pltpu.make_async_copy(wo, wo, sem_o.at[0]).wait()
    pltpu.make_async_copy(wd, wd, sem_f.at[0]).wait()
    cp_x.wait()
    pltpu.make_async_copy(wg, wg, sem_f.at[1]).wait()
    pltpu.make_async_copy(wu, wu, sem_f.at[2]).wait()

    row = lax.broadcasted_iota(jnp.int32, (2 * L, 2 * L), 0)
    col = lax.broadcasted_iota(jnp.int32, (2 * L, 2 * L), 1)
    same = (row >= L) == (col >= L)
    r_in = jnp.where(row >= L, row - L, row)
    c_in = jnp.where(col >= L, col - L, col)
    valid = same & ((r_in < M) | (r_in >= c_in))
    fill = jnp.where(same, jnp.float32(-1e9), jnp.float32(-jnp.inf))
    lo = lax.broadcasted_iota(jnp.int32, (L, 128), 1) < (Dh - 128)

    FC = F // NF

    def ffn_gu(hn, c):
        g = _mm(hn, wg[:, c * FC:(c + 1) * FC])
        u = _mm(hn, wu[:, c * FC:(c + 1) * FC])
        return (g * (1.0 / (1.0 + jnp.exp(-g))) * u).astype(BF16)

    def ffn_down(hprev, acts):
        y = hprev
        for c in range(NF):
            y = y + _mm(acts[c], wd[c * FC:(c + 1) * FC, :])
        return y

    OR = UNROLL * seg

    def ocopy(i):
        r = pl.ds(pl.multiple_of(i * OR, OR), OR)
        return pltpu.make_async_copy(out_v.at[r, :], out_hbm.at[r, :], sem_m.at[1])

    def lhs(mem, s):
        return jnp.concatenate([mem, _ln(x_v[s, PR:, :].astype(F32))], axis=0).astype(BF16)

    def step(s, hin):
        rp = pl.multiple_of(jnp.maximum(s - 1, 0) * seg, seg)
        rq = pl.multiple_of(s * PR, PR)
        hprev = h_v[...]
        hn = _ln(hprev).astype(BF16)
        st = {}

        def A(j):
            y = _mm(hin, pltpu.bitcast(wqkv[j], BF16))
            st['qkv', j] = jnp.concatenate([y[:M], pre[j, pl.ds(rq, PR), :], y[M:]], axis=0)

        def QK(j):
            y = st.pop(('qkv', j))
            t = [y[:, i * 128:(i + 1) * 128] for i in range(9)]
            qm = jnp.concatenate([t[0], t[2]], axis=0)
            km = jnp.concatenate([t[3], t[5]], axis=0).astype(BF16)
            kt = jnp.concatenate([jnp.where(lo, t[4], 0.0), jnp.where(lo, 0.0, t[4])], axis=0).astype(BF16)
            st['vm', j] = jnp.concatenate([t[6], t[8]], axis=0).astype(BF16)
            st['vt', j] = jnp.concatenate([jnp.where(lo, t[7], 0.0), jnp.where(lo, 0.0, t[7])], axis=0).astype(BF16)
            sm = _mm_nt(qm, km)
            stl = _mm_nt(t[1], kt)
            sc = (sm + jnp.concatenate([stl, stl], axis=0)) * scale
            sc = jnp.where(valid, sc, fill)
            mx = jnp.max(sc, axis=-1, keepdims=True)
            e = jnp.exp(sc - mx)
            p = e / jnp.sum(e, axis=-1, keepdims=True)
            st['p', j] = p

        def PV(j):
            p = st.pop(('p', j))
            om = _mm(p, st.pop(('vm', j)))
            ot = _mm(p[:L] + p[L:], st.pop(('vt', j)))
            st['o', j] = jnp.concatenate([om[:L], ot, om[L:]], axis=1)

        def C(j):
            y = _mm(st.pop(('o', j)), wo[j])
            st['acc'] = y if j == 0 else st['acc'] + y

        acts = []
        lq, lp, lc = LAG // 100, LAG // 10 % 10, LAG % 10
        for t in range(NP + lc):
            for op in PERMS[ORDER]:
                if op == 'A':
                    if t < NP:
                        A(t)
                    elif t - NP < NF:
                        acts.append(ffn_gu(hn, t - NP))
                elif op == 'C' and 0 <= t - lc < NP:
                    C(t - lc)
                elif op == 'P' and 0 <= t - lp < NP:
                    PV(t - lp)
                elif op == 'Q' and 0 <= t - lq < NP:
                    QK(t - lq)
        while len(acts) < NF:
            acts.append(ffn_gu(hn, len(acts)))
        out_v[pl.ds(rp, seg), :] = ffn_down(hprev, acts).astype(BF16)
        acc = st['acc']
        h_v[...] = x_v[s].astype(F32) + acc[M:]
        return lhs(acc[:M], jnp.minimum(s + 1, n_seg - 1))

    def steps(i, hin):
        @pl.when(i >= 2)
        def _():
            ocopy(i - 2).start()
        for u in range(UNROLL):
            hin = step(i * UNROLL + u, hin)
        return hin

    n_it = n_seg // UNROLL
    lax.fori_loop(0, n_it, steps, lhs(mem0_ref[...].astype(F32), 0))
    ocopy(n_it - 2).start()
    hprev = h_v[...]
    hn = _ln(hprev).astype(BF16)
    acts = [ffn_gu(hn, c) for c in range(NF)]
    out_v[S - seg:, :] = ffn_down(hprev, acts).astype(BF16)
    ocopy(n_it - 1).start()
    pltpu.make_async_copy(out_v, out_hbm, sem_m.at[1]).wait()


@functools.partial(jax.jit, static_argnames=("A_seg_len",))
def pallas_sequential_preLN__memory_aug_recurrent_mem_tr__swiglu_ffn__prompt_kernel(A_x, A_mem0, A_Wq, A_Wk, A_Wv, A_Wo, A_seg_len, B_x, B_w_gate, B_w_up, B_w_down):
    B, S, Dm = A_x.shape
    _, H, Dh = A_Wq.shape
    M = A_mem0.shape[1]
    F = B_w_gate.shape[1]
    seg = A_seg_len
    NP, PW = H // 2, 2 * Dh
    n_seg = S // seg
    wt = lambda w: jnp.transpose(w, (1, 2, 0)).reshape(H * Dh, Dm)
    anyspec = pl.BlockSpec(memory_space=pl.ANY)
    out = pl.pallas_call(
        functools.partial(_kernel, S=S, Dm=Dm, H=H, Dh=Dh, M=M, seg=seg, F=F),
        out_shape=jax.ShapeDtypeStruct((S, Dm), A_x.dtype),
        in_specs=[anyspec, pl.BlockSpec(memory_space=pltpu.VMEM)] + [anyspec] * 7,
        out_specs=anyspec,
        scratch_shapes=[
            pltpu.VMEM((n_seg, seg, Dm), BF16),
            pltpu.VMEM((n_seg, M, Dm), BF16),
            pltpu.VMEM((n_seg * M, Dm), BF16),
            pltpu.VMEM((NP, n_seg * M, 3 * PW), F32),
            pltpu.VMEM((seg, Dm), F32),
            pltpu.VMEM((S, Dm), BF16),
            pltpu.VMEM((RING, 3, PW, Dm), BF16),
            pltpu.VMEM((NP, Dm // 2, 3 * PW), U32),
            pltpu.VMEM((NP, PW, Dm), BF16),
            pltpu.VMEM((Dm, F), BF16),
            pltpu.VMEM((Dm, F), BF16),
            pltpu.VMEM((F, Dm), BF16),
            pltpu.SemaphoreType.DMA((RING * 3,)),
            pltpu.SemaphoreType.DMA((1,)),
            pltpu.SemaphoreType.DMA((3,)),
            pltpu.SemaphoreType.DMA((3,)),
        ],
        compiler_params=pltpu.CompilerParams(vmem_limit_bytes=110 << 20, disable_bounds_checks=True,
            flags={'XLA_TPU_EVENLY_DISTRIBUTE_CRITICAL_NODES': True}),
    )(A_x.reshape(n_seg, seg, Dm), A_mem0.reshape(M, Dm), wt(A_Wq), wt(A_Wk), wt(A_Wv),
      A_Wo.reshape(H * Dh, Dm), B_w_gate, B_w_up, B_w_down)
    return out.reshape(B, S, Dm)
```

```python
import functools
import itertools
import numpy as np
import jax
import jax.numpy as jnp
from jax import lax
import jax.experimental.pallas as pl
import jax.experimental.pallas.tpu as pltpu

F32 = jnp.float32
BF16 = jnp.bfloat16
U32 = jnp.uint32
RING = 4
PERMS = [a + ''.join(p) for a in 'A' for p in itertools.permutations('CPQ')]
ORDER = 1
LAG = 134
NF = 4
UNROLL = 3


def _mm(a, b):
    return lax.dot_general(a, b, (((1,), (0,)), ((), ())), preferred_element_type=F32)


def _mm_nt(a, b):
    return lax.dot_general(a, b, (((1,), (1,)), ((), ())), preferred_element_type=F32)


def _ln(x):
    m = jnp.mean(x, axis=-1, keepdims=True)
    d = x - m
    v = jnp.mean(d * d, axis=-1, keepdims=True)
    return d * lax.rsqrt(v + 1e-5)


def _kernel(x_hbm, mem0_ref, wq_hbm, wk_hbm, wv_hbm, wo_hbm, wg_hbm, wu_hbm, wd_hbm,
            out_hbm,
            x_v, xq_v, xp_v, pre, h_v, out_v, stg, wqkv, wo, wg, wu, wd, sem_w, sem_o, sem_f, sem_m,
            *, S, Dm, H, Dh, M, seg, F):
    NP = H // 2
    PW = 2 * Dh
    L = M + seg
    n_seg = S // seg
    scale = Dh ** (-0.5)
    PR = M
    GR = 48
    NG = -(-Dm // GR)

    def wcopies(j):
        slot = j % RING
        return [pltpu.make_async_copy(src.at[pl.ds(j * PW, PW), :], stg.at[slot, i], sem_w.at[slot * 3 + i])
                for i, src in enumerate((wq_hbm, wk_hbm, wv_hbm))]

    cp_p = pltpu.make_async_copy(x_hbm.at[:, pl.ds(0, PR), :], xq_v, sem_m.at[2])
    cp_x = pltpu.make_async_copy(x_hbm, x_v, sem_m.at[0])
    cp_p.start()
    wcopies(0)[0].start()
    cp_p.wait()
    for c in wcopies(0)[1:]:
        c.start()
    for i in range(n_seg * PR // 128):
        xs = jnp.concatenate([xq_v[i * (128 // PR) + t].astype(F32) for t in range(128 // PR)], axis=0)
        xp_v[i * 128:(i + 1) * 128, :] = _ln(xs).astype(BF16)

    def transpose_w(j, i):
        slot = j % RING
        for t in range(PW // 128):
            blk = stg[slot, i, t * 128:(t + 1) * 128, :]
            wqkv[j, :, i * PW + t * 128:i * PW + (t + 1) * 128] = pltpu.bitcast(
                blk.astype(F32).T.astype(BF16), U32)

    def transpose_pair(j):
        for i in range(3):
            transpose_w(j, i)

    def project_pre(j, c0=0, c1=3 * PW):
        w = pltpu.bitcast(wqkv[j, :, c0:c1], BF16)
        for c in range(n_seg * PR // 128):
            pre[j, c * 128:(c + 1) * 128, c0:c1] = _mm(xp_v[c * 128:(c + 1) * 128, :], w)

    OB = H * Dh // NP
    DB = F // NP

    GB = Dm // NP

    def side_copies(j):
        return [pltpu.make_async_copy(wo_hbm.at[pl.ds(j * OB, OB), :], wo.at[j], sem_o.at[0]),
                pltpu.make_async_copy(wd_hbm.at[pl.ds(j * DB, DB), :], wd.at[pl.ds(j * DB, DB), :], sem_f.at[0]),
                pltpu.make_async_copy(wg_hbm.at[pl.ds(j * GB, GB), :], wg.at[pl.ds(j * GB, GB), :], sem_f.at[1]),
                pltpu.make_async_copy(wu_hbm.at[pl.ds(j * GB, GB), :], wu.at[pl.ds(j * GB, GB), :], sem_f.at[2])]

    w0 = wcopies(0)
    w0[0].wait()
    for c in wcopies(1):
        c.start()
    transpose_w(0, 0)
    project_pre(0, 0, PW)
    w0[1].wait()
    w0[2].wait()
    for j in range(2, RING):
        for c in wcopies(j):
            c.start()
    transpose_w(0, 1)
    transpose_w(0, 2)
    project_pre(0, PW, 2 * PW)
    for c in wcopies(1):
        c.wait()
    for c in wcopies(RING) + side_copies(0) + [cp_x]:
        c.start()
    transpose_pair(1)
    project_pre(0, 2 * PW, 3 * PW)

    def pro_body(j, c, refill):
        for cp in wcopies(j + 1):
            cp.wait()
        if refill:
            for cp in wcopies(j + RING):
                cp.start()
        for cp in side_copies(j):
            cp.start()
        transpose_pair(j + 1)
        project_pre(j)
        return c
    lax.fori_loop(1, NP - RING, functools.partial(pro_body, refill=True), 0)
    lax.fori_loop(NP - RING, NP - 1, functools.partial(pro_body, refill=False), 0)
    for cp in side_copies(NP - 1):
        cp.start()
    project_pre(NP - 1)
    pltpu.make_async_copy(wo, wo, sem_o.at[0]).wait()
    pltpu.make_async_copy(wd, wd, sem_f.at[0]).wait()
    cp_x.wait()
    pltpu.make_async_copy(wg, wg, sem_f.at[1]).wait()
    pltpu.make_async_copy(wu, wu, sem_f.at[2]).wait()

    row = lax.broadcasted_iota(jnp.int32, (2 * L, 2 * L), 0)
    col = lax.broadcasted_iota(jnp.int32, (2 * L, 2 * L), 1)
    same = (row >= L) == (col >= L)
    r_in = jnp.where(row >= L, row - L, row)
    c_in = jnp.where(col >= L, col - L, col)
    valid = same & ((r_in < M) | (r_in >= c_in))
    fill = jnp.where(same, jnp.float32(-1e9), jnp.float32(-jnp.inf))
    lo = lax.broadcasted_iota(jnp.int32, (L, 128), 1) < (Dh - 128)

    FC = F // NF

    def ffn_gu(hn, c):
        g = _mm(hn, wg[:, c * FC:(c + 1) * FC])
        u = _mm(hn, wu[:, c * FC:(c + 1) * FC])
        return (g * (1.0 / (1.0 + jnp.exp(-g))) * u).astype(BF16)

    def ffn_down(hprev, acts):
        y = hprev
        for c in range(NF):
            y = y + _mm(acts[c], wd[c * FC:(c + 1) * FC, :])
        return y

    OR = UNROLL * seg

    def ocopy(i):
        r = pl.ds(pl.multiple_of(i * OR, OR), OR)
        return pltpu.make_async_copy(out_v.at[r, :], out_hbm.at[r, :], sem_m.at[1])

    def lhs(mem, s):
        return jnp.concatenate([mem, _ln(x_v[s, PR:, :].astype(F32))], axis=0).astype(BF16)

    def step(s, hin, first=False):
        rq = 0 if first else pl.multiple_of(s * PR, PR)
        if not first:
            hprev = h_v[...]
            hn = _ln(hprev).astype(BF16)
        st = {}

        def A(j):
            y = _mm(hin, pltpu.bitcast(wqkv[j], BF16))
            st['qkv', j] = jnp.concatenate([y[:M], pre[j, pl.ds(rq, PR), :], y[M:]], axis=0)

        def QK(j):
            y = st.pop(('qkv', j))
            t = [y[:, i * 128:(i + 1) * 128] for i in range(9)]
            qm = jnp.concatenate([t[0], t[2]], axis=0)
            km = jnp.concatenate([t[3], t[5]], axis=0).astype(BF16)
            kt = jnp.concatenate([jnp.where(lo, t[4], 0.0), jnp.where(lo, 0.0, t[4])], axis=0).astype(BF16)
            st['vm', j] = jnp.concatenate([t[6], t[8]], axis=0).astype(BF16)
            st['vt', j] = jnp.concatenate([jnp.where(lo, t[7], 0.0), jnp.where(lo, 0.0, t[7])], axis=0).astype(BF16)
            sm = _mm_nt(qm, km)
            stl = _mm_nt(t[1], kt)
            sc = (sm + jnp.concatenate([stl, stl], axis=0)) * scale
            sc = jnp.where(valid, sc, fill)
            mx = jnp.max(sc, axis=-1, keepdims=True)
            e = jnp.exp(sc - mx)
            p = e / jnp.sum(e, axis=-1, keepdims=True)
            st['p', j] = p

        def PV(j):
            p = st.pop(('p', j))
            om = _mm(p, st.pop(('vm', j)))
            ot = _mm(p[:L] + p[L:], st.pop(('vt', j)))
            st['o', j] = jnp.concatenate([om[:L], ot, om[L:]], axis=1)

        def C(j):
            y = _mm(st.pop(('o', j)), wo[j])
            st['acc'] = y if j == 0 else st['acc'] + y

        acts = []
        lq, lp, lc = LAG // 100, LAG // 10 % 10, LAG % 10
        for t in range(NP + lc):
            for op in PERMS[ORDER]:
                if op == 'A':
                    if t < NP:
                        A(t)
                    elif t - NP < NF and not first:
                        acts.append(ffn_gu(hn, t - NP))
                elif op == 'C' and 0 <= t - lc < NP:
                    C(t - lc)
                elif op == 'P' and 0 <= t - lp < NP:
                    PV(t - lp)
                elif op == 'Q' and 0 <= t - lq < NP:
                    QK(t - lq)
        if not first:
            while len(acts) < NF:
                acts.append(ffn_gu(hn, len(acts)))
            rp = pl.multiple_of((s - 1) * seg, seg)
            out_v[pl.ds(rp, seg), :] = ffn_down(hprev, acts).astype(BF16)
        acc = st['acc']
        h_v[...] = x_v[s].astype(F32) + acc[M:]
        return lhs(acc[:M], jnp.minimum(s + 1, n_seg - 1))

    def steps(i, hin):
        @pl.when(i >= 1)
        def _():
            ocopy(i - 1).start()
        for u in range(UNROLL):
            hin = step(1 + i * UNROLL + u, hin)
        return hin

    n_it = (n_seg - 1) // UNROLL
    assert n_it * UNROLL == n_seg - 1
    lax.fori_loop(0, n_it, steps, step(0, lhs(mem0_ref[...].astype(F32), 0), first=True))
    ocopy(n_it - 1).start()
    hprev = h_v[...]
    hn = _ln(hprev).astype(BF16)
    acts = [ffn_gu(hn, c) for c in range(NF)]
    out_v[S - seg:, :] = ffn_down(hprev, acts).astype(BF16)
    pltpu.make_async_copy(out_v.at[pl.ds(S - seg, seg), :], out_hbm.at[pl.ds(S - seg, seg), :], sem_m.at[1]).start()
    pltpu.make_async_copy(out_v, out_hbm, sem_m.at[1]).wait()


@functools.partial(jax.jit, static_argnames=("A_seg_len",))
def pallas_sequential_preLN__memory_aug_recurrent_mem_tr__swiglu_ffn__prompt_kernel(A_x, A_mem0, A_Wq, A_Wk, A_Wv, A_Wo, A_seg_len, B_x, B_w_gate, B_w_up, B_w_down):
    B, S, Dm = A_x.shape
    _, H, Dh = A_Wq.shape
    M = A_mem0.shape[1]
    F = B_w_gate.shape[1]
    seg = A_seg_len
    NP, PW = H // 2, 2 * Dh
    n_seg = S // seg
    wt = lambda w: jnp.transpose(w, (1, 2, 0)).reshape(H * Dh, Dm)
    anyspec = pl.BlockSpec(memory_space=pl.ANY)
    out = pl.pallas_call(
        functools.partial(_kernel, S=S, Dm=Dm, H=H, Dh=Dh, M=M, seg=seg, F=F),
        out_shape=jax.ShapeDtypeStruct((S, Dm), A_x.dtype),
        in_specs=[anyspec, pl.BlockSpec(memory_space=pltpu.VMEM)] + [anyspec] * 7,
        out_specs=anyspec,
        scratch_shapes=[
            pltpu.VMEM((n_seg, seg, Dm), BF16),
            pltpu.VMEM((n_seg, M, Dm), BF16),
            pltpu.VMEM((n_seg * M, Dm), BF16),
            pltpu.VMEM((NP, n_seg * M, 3 * PW), F32),
            pltpu.VMEM((seg, Dm), F32),
            pltpu.VMEM((S, Dm), BF16),
            pltpu.VMEM((RING, 3, PW, Dm), BF16),
            pltpu.VMEM((NP, Dm // 2, 3 * PW), U32),
            pltpu.VMEM((NP, PW, Dm), BF16),
            pltpu.VMEM((Dm, F), BF16),
            pltpu.VMEM((Dm, F), BF16),
            pltpu.VMEM((F, Dm), BF16),
            pltpu.SemaphoreType.DMA((RING * 3,)),
            pltpu.SemaphoreType.DMA((1,)),
            pltpu.SemaphoreType.DMA((3,)),
            pltpu.SemaphoreType.DMA((3,)),
        ],
        compiler_params=pltpu.CompilerParams(vmem_limit_bytes=110 << 20, disable_bounds_checks=True,
            flags={'XLA_TPU_EVENLY_DISTRIBUTE_CRITICAL_NODES': True}),
    )(A_x.reshape(n_seg, seg, Dm), A_mem0.reshape(M, Dm), wt(A_Wq), wt(A_Wk), wt(A_Wv),
      A_Wo.reshape(H * Dh, Dm), B_w_gate, B_w_up, B_w_down)
    return out.reshape(B, S, Dm)
```

```python
import functools
import itertools
import numpy as np
import jax
import jax.numpy as jnp
from jax import lax
import jax.experimental.pallas as pl
import jax.experimental.pallas.tpu as pltpu

F32 = jnp.float32
BF16 = jnp.bfloat16
U32 = jnp.uint32
RING = 4
PEEL = 1
START = 1
FLAG = 1
ONE = 1
UW = 0
CH = 128
PERMS = [a + ''.join(p) for a in 'A' for p in itertools.permutations('CPQ')]
ORDER = 1
LAG = 134
NF = 4
UNROLL = 3


def _mm(a, b):
    return lax.dot_general(a, b, (((1,), (0,)), ((), ())), preferred_element_type=F32)


def _mm_nt(a, b):
    return lax.dot_general(a, b, (((1,), (1,)), ((), ())), preferred_element_type=F32)


def _ln(x):
    m = jnp.mean(x, axis=-1, keepdims=True)
    d = x - m
    v = jnp.mean(d * d, axis=-1, keepdims=True)
    return d * lax.rsqrt(v + 1e-5)


def _kernel(x_hbm, mem0_ref, wq_hbm, wk_hbm, wv_hbm, wo_hbm, wg_hbm, wu_hbm, wd_hbm,
            out_hbm,
            x_v, xq_v, xp_v, pre, h_v, out_v, stg, wqkv, wo, wg, wu, wd, sem_w, sem_o, sem_f, sem_m,
            *, S, Dm, H, Dh, M, seg, F):
    NP = H // 2
    PW = 2 * Dh
    L = M + seg
    n_seg = S // seg
    scale = Dh ** (-0.5)
    PR = M
    GR = 48
    NG = -(-Dm // GR)

    def wcopies(j):
        slot = j % RING
        return [pltpu.make_async_copy(src.at[pl.ds(j * PW, PW), :], stg.at[slot, i], sem_w.at[slot * 3 + i])
                for i, src in enumerate((wq_hbm, wk_hbm, wv_hbm))]

    cp_p = pltpu.make_async_copy(x_hbm.at[:, pl.ds(0, PR), :], xq_v, sem_m.at[2])
    cp_x = pltpu.make_async_copy(x_hbm, x_v, sem_m.at[0])
    cp_p.start()
    wcopies(0)[0].start()
    cp_p.wait()
    for c in wcopies(0)[1:]:
        c.start()
    for i in range(n_seg * PR // 128):
        xs = jnp.concatenate([xq_v[i * (128 // PR) + t].astype(F32) for t in range(128 // PR)], axis=0)
        xp_v[i * 128:(i + 1) * 128, :] = _ln(xs).astype(BF16)

    def transpose_w(j, i):
        slot = j % RING
        for t in range(PW // 128):
            blk = stg[slot, i, t * 128:(t + 1) * 128, :]
            wqkv[j, :, i * PW + t * 128:i * PW + (t + 1) * 128] = pltpu.bitcast(
                blk.astype(F32).T.astype(BF16), U32)

    def transpose_pair(j):
        for i in range(3):
            transpose_w(j, i)

    def project_pre(j, c0=0, c1=3 * PW):
        w = pltpu.bitcast(wqkv[j, :, c0:c1], BF16)
        for c in range(n_seg * PR // CH):
            pre[j, c * CH:(c + 1) * CH, c0:c1] = _mm(xp_v[c * CH:(c + 1) * CH, :], w)

    N1 = NP - RING
    OB = H * Dh // N1
    DB = F // N1

    def side_copies(j):
        k = 2 if UW == 1 else 1
        ro = pl.ds(pl.multiple_of(j * (OB // k), OB // k), OB // k)
        rd = pl.ds(pl.multiple_of(j * (DB // k), DB // k), DB // k)
        rf = pl.ds(pl.multiple_of(j * DB, DB), DB)
        bc = (lambda r: r.bitcast(U32)) if UW == 1 else (lambda r: r)
        return [pltpu.make_async_copy(bc(wo_hbm).at[ro, :], wo.at[ro, :], sem_o.at[0]),
                pltpu.make_async_copy(bc(wd_hbm).at[rd, :], wd.at[rd, :], sem_f.at[0]),
                pltpu.make_async_copy(bc(wg_hbm).at[:, rf], wg.at[:, rf], sem_f.at[1]),
                pltpu.make_async_copy(bc(wu_hbm).at[:, rf], wu.at[:, rf], sem_f.at[2])]

    def wrows(ref, r0, r1):
        return pltpu.bitcast(ref[r0 // 2:r1 // 2, :], BF16) if UW else ref[r0:r1, :]

    def wcols(ref, c0, c1):
        return pltpu.bitcast(ref[:, c0:c1], BF16) if UW else ref[:, c0:c1]

    if START:
        w0 = wcopies(0)
        w0[0].wait()
        for c in wcopies(1):
            c.start()
        transpose_w(0, 0)
        project_pre(0, 0, PW)
        w0[1].wait()
        w0[2].wait()
        for j in range(2, RING):
            for c in wcopies(j):
                c.start()
        transpose_w(0, 1)
        transpose_w(0, 2)
        project_pre(0, PW, 2 * PW)
        for c in wcopies(1):
            c.wait()
        for c in wcopies(RING) + side_copies(0) + [cp_x]:
            c.start()
        transpose_pair(1)
        project_pre(0, 2 * PW, 3 * PW)
    else:
        for c in wcopies(0):
            c.wait()
        for j in range(1, RING):
            for c in wcopies(j):
                c.start()
        cp_x.start()
        transpose_pair(0)

    def pro_body(j, c, refill):
        if ONE:
            @pl.when(j < NP - 1)
            def _():
                for cp in wcopies(j + 1):
                    cp.wait()

            @pl.when(j < N1)
            def _():
                for cp in wcopies(j + RING) + side_copies(j):
                    cp.start()
        else:
            for cp in wcopies(j + 1):
                cp.wait()
            if refill:
                for cp in wcopies(j + RING) + side_copies(j):
                    cp.start()
        transpose_pair(j + 1)
        project_pre(j)
        return c
    if ONE:
        lax.fori_loop(START, NP, functools.partial(pro_body, refill=True), 0)
    else:
        lax.fori_loop(START, NP - RING, functools.partial(pro_body, refill=True), 0)
        lax.fori_loop(NP - RING, NP - 1, functools.partial(pro_body, refill=False), 0)
        project_pre(NP - 1)
    pltpu.make_async_copy(wo, wo, sem_o.at[0]).wait()
    pltpu.make_async_copy(wd, wd, sem_f.at[0]).wait()
    cp_x.wait()
    pltpu.make_async_copy(wg, wg, sem_f.at[1]).wait()
    pltpu.make_async_copy(wu, wu, sem_f.at[2]).wait()

    row = lax.broadcasted_iota(jnp.int32, (2 * L, 2 * L), 0)
    col = lax.broadcasted_iota(jnp.int32, (2 * L, 2 * L), 1)
    same = (row >= L) == (col >= L)
    r_in = jnp.where(row >= L, row - L, row)
    c_in = jnp.where(col >= L, col - L, col)
    valid = same & ((r_in < M) | (r_in >= c_in))
    fill = jnp.where(same, jnp.float32(-1e9), jnp.float32(-jnp.inf))
    lo = lax.broadcasted_iota(jnp.int32, (L, 128), 1) < (Dh - 128)

    FC = F // NF

    def ffn_gu(hn, c):
        g = _mm(hn, wcols(wg, c * FC, (c + 1) * FC))
        u = _mm(hn, wcols(wu, c * FC, (c + 1) * FC))
        return (g * (1.0 / (1.0 + jnp.exp(-g))) * u).astype(BF16)

    def ffn_down(hprev, acts):
        y = hprev
        for c in range(NF):
            y = y + _mm(acts[c], wrows(wd, c * FC, (c + 1) * FC))
        return y

    OR = UNROLL * seg

    def ocopy(i):
        r = pl.ds(pl.multiple_of(i * OR, OR), OR)
        return pltpu.make_async_copy(out_v.at[r, :], out_hbm.at[r, :], sem_m.at[1])

    def lhs(mem, s):
        return jnp.concatenate([mem, _ln(x_v[s, PR:, :].astype(F32))], axis=0).astype(BF16)

    def step(s, hin, first=False):
        rq = 0 if first else pl.multiple_of(s * PR, PR)
        if not first:
            hprev = h_v[...]
            hn = _ln(hprev).astype(BF16)
        st = {}

        def A(j):
            y = _mm(hin, pltpu.bitcast(wqkv[j], BF16))
            st['qkv', j] = jnp.concatenate([y[:M], pre[j, pl.ds(rq, PR), :], y[M:]], axis=0)

        def QK(j):
            y = st.pop(('qkv', j))
            t = [y[:, i * 128:(i + 1) * 128] for i in range(9)]
            qm = jnp.concatenate([t[0], t[2]], axis=0)
            km = jnp.concatenate([t[3], t[5]], axis=0).astype(BF16)
            kt = jnp.concatenate([jnp.where(lo, t[4], 0.0), jnp.where(lo, 0.0, t[4])], axis=0).astype(BF16)
            st['vm', j] = jnp.concatenate([t[6], t[8]], axis=0).astype(BF16)
            st['vt', j] = jnp.concatenate([jnp.where(lo, t[7], 0.0), jnp.where(lo, 0.0, t[7])], axis=0).astype(BF16)
            sm = _mm_nt(qm, km)
            stl = _mm_nt(t[1], kt)
            sc = (sm + jnp.concatenate([stl, stl], axis=0)) * scale
            sc = jnp.where(valid, sc, fill)
            mx = jnp.max(sc, axis=-1, keepdims=True)
            e = jnp.exp(sc - mx)
            p = e / jnp.sum(e, axis=-1, keepdims=True)
            st['p', j] = p

        def PV(j):
            p = st.pop(('p', j))
            om = _mm(p, st.pop(('vm', j)))
            ot = _mm(p[:L] + p[L:], st.pop(('vt', j)))
            st['o', j] = jnp.concatenate([om[:L], ot, om[L:]], axis=1)

        def C(j):
            y = _mm(st.pop(('o', j)), wrows(wo, j * PW, (j + 1) * PW))
            st['acc'] = y if j == 0 else st['acc'] + y

        acts = []
        lq, lp, lc = LAG // 100, LAG // 10 % 10, LAG % 10
        for t in range(NP + lc):
            for op in PERMS[ORDER]:
                if op == 'A':
                    if t < NP:
                        A(t)
                    elif t - NP < NF and not first:
                        acts.append(ffn_gu(hn, t - NP))
                elif op == 'C' and 0 <= t - lc < NP:
                    C(t - lc)
                elif op == 'P' and 0 <= t - lp < NP:
                    PV(t - lp)
                elif op == 'Q' and 0 <= t - lq < NP:
                    QK(t - lq)
        if not first:
            while len(acts) < NF:
                acts.append(ffn_gu(hn, len(acts)))
            rp = pl.multiple_of((s - 1 if PEEL else jnp.maximum(s - 1, 0)) * seg, seg)
            out_v[pl.ds(rp, seg), :] = ffn_down(hprev, acts).astype(BF16)
        acc = st['acc']
        h_v[...] = x_v[s].astype(F32) + acc[M:]
        return lhs(acc[:M], jnp.minimum(s + 1, n_seg - 1))

    def steps(i, hin):
        @pl.when(i >= 2 - PEEL)
        def _():
            ocopy(i - 2 + PEEL).start()
        for u in range(UNROLL):
            hin = step(PEEL + i * UNROLL + u, hin)
        return hin

    n_it = (n_seg - PEEL) // UNROLL
    assert n_it * UNROLL == n_seg - PEEL
    hin0 = lhs(mem0_ref[...].astype(F32), 0)
    if PEEL:
        hin0 = step(0, hin0, first=True)
    else:
        h_v[...] = jnp.zeros(h_v.shape, F32)
    lax.fori_loop(0, n_it, steps, hin0)
    ocopy(n_it - 2 + PEEL).start()
    hprev = h_v[...]
    hn = _ln(hprev).astype(BF16)
    acts = [ffn_gu(hn, c) for c in range(NF)]
    out_v[S - seg:, :] = ffn_down(hprev, acts).astype(BF16)
    TR = seg if PEEL else OR
    pltpu.make_async_copy(out_v.at[pl.ds(S - TR, TR), :], out_hbm.at[pl.ds(S - TR, TR), :], sem_m.at[1]).start()
    pltpu.make_async_copy(out_v, out_hbm, sem_m.at[1]).wait()


@functools.partial(jax.jit, static_argnames=("A_seg_len",))
def pallas_sequential_preLN__memory_aug_recurrent_mem_tr__swiglu_ffn__prompt_kernel(A_x, A_mem0, A_Wq, A_Wk, A_Wv, A_Wo, A_seg_len, B_x, B_w_gate, B_w_up, B_w_down):
    B, S, Dm = A_x.shape
    _, H, Dh = A_Wq.shape
    M = A_mem0.shape[1]
    F = B_w_gate.shape[1]
    seg = A_seg_len
    NP, PW = H // 2, 2 * Dh
    n_seg = S // seg
    wt = lambda w: jnp.transpose(w, (1, 2, 0)).reshape(H * Dh, Dm)
    wbuf = lambda r, c: pltpu.VMEM((r // 2, c), U32) if UW else pltpu.VMEM((r, c), BF16)
    anyspec = pl.BlockSpec(memory_space=pl.ANY)
    out = pl.pallas_call(
        functools.partial(_kernel, S=S, Dm=Dm, H=H, Dh=Dh, M=M, seg=seg, F=F),
        out_shape=jax.ShapeDtypeStruct((S, Dm), A_x.dtype),
        in_specs=[anyspec, pl.BlockSpec(memory_space=pltpu.VMEM)] + [anyspec] * 7,
        out_specs=anyspec,
        scratch_shapes=[
            pltpu.VMEM((n_seg, seg, Dm), BF16),
            pltpu.VMEM((n_seg, M, Dm), BF16),
            pltpu.VMEM((n_seg * M, Dm), BF16),
            pltpu.VMEM((NP, n_seg * M, 3 * PW), F32),
            pltpu.VMEM((seg, Dm), F32),
            pltpu.VMEM((S, Dm), BF16),
            pltpu.VMEM((RING, 3, PW, Dm), BF16),
            pltpu.VMEM((NP + ONE, Dm // 2, 3 * PW), U32),
            wbuf(H * Dh, Dm), wbuf(Dm, F), wbuf(Dm, F), wbuf(F, Dm),
            pltpu.SemaphoreType.DMA((RING * 3,)),
            pltpu.SemaphoreType.DMA((1,)),
            pltpu.SemaphoreType.DMA((3,)),
            pltpu.SemaphoreType.DMA((3,)),
        ],
        compiler_params=pltpu.CompilerParams(vmem_limit_bytes=110 << 20, disable_bounds_checks=True,
            flags={'XLA_TPU_EVENLY_DISTRIBUTE_CRITICAL_NODES': bool(FLAG)}),
    )(A_x.reshape(n_seg, seg, Dm), A_mem0.reshape(M, Dm), wt(A_Wq), wt(A_Wk), wt(A_Wv),
      A_Wo.reshape(H * Dh, Dm), B_w_gate, B_w_up, B_w_down)
    return out.reshape(B, S, Dm)
```

```python
import functools

import jax
import jax.numpy as jnp
from jax import lax
import jax.experimental.pallas as pl
import jax.experimental.pallas.tpu as pltpu

F32 = jnp.float32
BF16 = jnp.bfloat16
U32 = jnp.uint32

LANES = 128
RING = 4
UNROLL = 3
NF = 4
LAG_QK, LAG_PV, LAG_WO = 1, 3, 4


def _mm(a, b):
    return lax.dot_general(a, b, (((1,), (0,)), ((), ())), preferred_element_type=F32)


def _mm_nt(a, b):
    return lax.dot_general(a, b, (((1,), (1,)), ((), ())), preferred_element_type=F32)


def _ln(x):
    m = jnp.mean(x, axis=-1, keepdims=True)
    d = x - m
    v = jnp.mean(d * d, axis=-1, keepdims=True)
    return d * lax.rsqrt(v + 1e-5)


def _body(x_hbm, mem0_ref, wq_hbm, wk_hbm, wv_hbm, wo_hbm, wg_hbm, wu_hbm, wd_hbm,
          out_hbm,
          x_v, xq_v, xp_v, pre, h_v, out_v, stg, wqkv, wo, wg, wu, wd,
          sem_w, sem_o, sem_f, sem_m,
          *, S, Dm, H, Dh, M, seg, F):
    NP = H // 2
    PW = 2 * Dh
    L = M + seg
    n_seg = S // seg
    scale = Dh ** (-0.5)
    PR = M
    NC = n_seg * PR // LANES
    N1 = NP - RING
    OB = H * Dh // N1
    FB = F // N1
    FC = F // NF

    def wcopies(j):
        slot = j % RING
        return [pltpu.make_async_copy(src.at[pl.ds(j * PW, PW), :], stg.at[slot, i],
                                      sem_w.at[slot * 3 + i])
                for i, src in enumerate((wq_hbm, wk_hbm, wv_hbm))]

    def side_copies(j):
        ro = pl.ds(pl.multiple_of(j * OB, OB), OB)
        rf = pl.ds(pl.multiple_of(j * FB, FB), FB)
        return [pltpu.make_async_copy(wo_hbm.at[ro, :], wo.at[ro, :], sem_o.at[0]),
                pltpu.make_async_copy(wd_hbm.at[rf, :], wd.at[rf, :], sem_f.at[0]),
                pltpu.make_async_copy(wg_hbm.at[:, rf], wg.at[:, rf], sem_f.at[1]),
                pltpu.make_async_copy(wu_hbm.at[:, rf], wu.at[:, rf], sem_f.at[2])]

    OR = UNROLL * seg

    def ocopy(i):
        r = pl.ds(pl.multiple_of(i * OR, OR), OR)
        return pltpu.make_async_copy(out_v.at[r, :], out_hbm.at[r, :], sem_m.at[1])

    def ln_pre(c):
        n = LANES // PR
        xs = jnp.concatenate([xq_v[c * n + t].astype(F32) for t in range(n)], axis=0)
        xp_v[c * LANES:(c + 1) * LANES, :] = _ln(xs).astype(BF16)

    def transpose_w(j, i):
        for t in range(PW // LANES):
            blk = stg[j % RING, i, t * LANES:(t + 1) * LANES, :]
            c0 = i * PW + t * LANES
            wqkv[j, :, c0:c0 + LANES] = pltpu.bitcast(blk.astype(F32).T.astype(BF16), U32)

    def transpose_pair(j):
        for i in range(3):
            transpose_w(j, i)

    def project_pre(j, c0=0, c1=3 * PW, chunks=range(NC)):
        w = pltpu.bitcast(wqkv[j, :, c0:c1], BF16)
        for c in chunks:
            rows = slice(c * LANES, (c + 1) * LANES)
            pre[j, rows, c0:c1] = _mm(xp_v[rows, :], w)

    cp_p = pltpu.make_async_copy(x_hbm.at[:, pl.ds(0, PR), :], xq_v, sem_m.at[2])
    cp_x = pltpu.make_async_copy(x_hbm, x_v, sem_m.at[0])
    w0 = wcopies(0)
    cp_p.start()
    w0[0].start()
    cp_p.wait()
    w0[1].start()
    w0[2].start()
    w0[0].wait()
    for cp in wcopies(1):
        cp.start()
    transpose_w(0, 0)
    for c in range(NC):
        ln_pre(c)
    project_pre(0, 0, PW)
    w0[1].wait()
    w0[2].wait()
    for j in range(2, RING):
        for cp in wcopies(j):
            cp.start()
    transpose_w(0, 1)
    transpose_w(0, 2)
    project_pre(0, PW, 2 * PW)
    for cp in wcopies(1):
        cp.wait()
    for cp in wcopies(RING) + side_copies(0) + [cp_x]:
        cp.start()
    transpose_pair(1)
    project_pre(0, 2 * PW, 3 * PW)

    def pro_body(i, carry):
        j = i + 1
        for cp in wcopies(j + 1):
            cp.wait()

        @pl.when(j < N1)
        def _():
            for cp in wcopies(j + RING) + side_copies(j):
                cp.start()

        transpose_pair(j + 1)
        project_pre(j)
        return carry

    lax.fori_loop(0, NP - 2, pro_body, 0)
    pltpu.make_async_copy(wo, wo, sem_o.at[0]).wait()
    pltpu.make_async_copy(wd, wd, sem_f.at[0]).wait()
    cp_x.wait()
    pltpu.make_async_copy(wg, wg, sem_f.at[1]).wait()
    pltpu.make_async_copy(wu, wu, sem_f.at[2]).wait()

    row = lax.broadcasted_iota(jnp.int32, (2 * L, 2 * L), 0)
    col = lax.broadcasted_iota(jnp.int32, (2 * L, 2 * L), 1)
    same_head = (row >= L) == (col >= L)
    r_in = jnp.where(row >= L, row - L, row)
    c_in = jnp.where(col >= L, col - L, col)
    valid = same_head & ((r_in < M) | (r_in >= c_in))
    fill = jnp.where(same_head, jnp.float32(-1e9), jnp.float32(-jnp.inf))
    lo = lax.broadcasted_iota(jnp.int32, (L, LANES), 1) < (Dh - LANES)

    def split_shared(t):
        return jnp.concatenate([jnp.where(lo, t, 0.0), jnp.where(lo, 0.0, t)], axis=0).astype(BF16)

    def ffn_gate_up(hn, c):
        g = _mm(hn, wg[:, c * FC:(c + 1) * FC])
        u = _mm(hn, wu[:, c * FC:(c + 1) * FC])
        return (g * (1.0 / (1.0 + jnp.exp(-g))) * u).astype(BF16)

    def ffn_down(h, acts):
        for c in range(NF):
            h = h + _mm(acts[c], wd[c * FC:(c + 1) * FC, :])
        return h

    def step_input(mem, s):
        return jnp.concatenate([mem, _ln(x_v[s, PR:, :].astype(F32))], axis=0).astype(BF16)

    def step(s, hin, first=False):
        rq = 0 if first else pl.multiple_of(s * PR, PR)
        if not first:
            h_prev = h_v[...]
            hn = _ln(h_prev).astype(BF16)
        st = {}
        acts = []

        def project(j):
            y = _mm(hin, pltpu.bitcast(wqkv[j], BF16))
            st["qkv", j] = jnp.concatenate([y[:M], pre[j, pl.ds(rq, PR), :], y[M:]], axis=0)

        def scores(j):
            y = st.pop(("qkv", j))
            t = [y[:, i * LANES:(i + 1) * LANES] for i in range(9)]
            qm = jnp.concatenate([t[0], t[2]], axis=0)
            km = jnp.concatenate([t[3], t[5]], axis=0).astype(BF16)
            kt = split_shared(t[4])
            st["vm", j] = jnp.concatenate([t[6], t[8]], axis=0).astype(BF16)
            st["vt", j] = split_shared(t[7])
            sm = _mm_nt(qm, km)
            stl = _mm_nt(t[1], kt)
            sc = (sm + jnp.concatenate([stl, stl], axis=0)) * scale
            sc = jnp.where(valid, sc, fill)
            e = jnp.exp(sc - jnp.max(sc, axis=-1, keepdims=True))
            st["p", j] = e / jnp.sum(e, axis=-1, keepdims=True)

        def mix(j):
            p = st.pop(("p", j))
            om = _mm(p, st.pop(("vm", j)))
            ot = _mm(p[:L] + p[L:], st.pop(("vt", j)))
            st["o", j] = jnp.concatenate([om[:L], ot, om[L:]], axis=1)

        def out_proj(j):
            y = _mm(st.pop(("o", j)), wo[j * PW:(j + 1) * PW, :])
            st["acc"] = y if j == 0 else st["acc"] + y

        for t in range(NP + LAG_WO):
            if t < NP:
                project(t)
            elif t - NP < NF and not first:
                acts.append(ffn_gate_up(hn, t - NP))
            if first:
                c = {NP - 2: 0, NP + 1: 1, NP + 2: 2}.get(t)
                if c is not None:
                    project_pre(NP - 1, chunks=(c,))
            if 0 <= t - LAG_WO < NP:
                out_proj(t - LAG_WO)
            if 0 <= t - LAG_PV < NP:
                mix(t - LAG_PV)
            if 0 <= t - LAG_QK < NP:
                scores(t - LAG_QK)
        if first:
            project_pre(NP - 1, chunks=range(3, NC))
        else:
            rp = pl.multiple_of((s - 1) * seg, seg)
            out_v[pl.ds(rp, seg), :] = ffn_down(h_prev, acts).astype(BF16)
        acc = st["acc"]
        h_v[...] = x_v[s].astype(F32) + acc[M:]
        return step_input(acc[:M], jnp.minimum(s + 1, n_seg - 1))

    def steps(i, hin):
        @pl.when(i >= 1)
        def _():
            ocopy(i - 1).start()

        for u in range(UNROLL):
            hin = step(1 + i * UNROLL + u, hin)
        return hin

    n_it = (n_seg - 1) // UNROLL
    hin = step(0, step_input(mem0_ref[...].astype(F32), 0), first=True)
    lax.fori_loop(0, n_it, steps, hin)

    ocopy(n_it - 1).start()
    h_prev = h_v[...]
    hn = _ln(h_prev).astype(BF16)
    acts = [ffn_gate_up(hn, c) for c in range(NF)]
    last = pl.ds(S - seg, seg)
    out_v[last, :] = ffn_down(h_prev, acts).astype(BF16)
    pltpu.make_async_copy(out_v.at[last, :], out_hbm.at[last, :], sem_m.at[1]).start()
    pltpu.make_async_copy(out_v, out_hbm, sem_m.at[1]).wait()


@functools.partial(jax.jit, static_argnames=("A_seg_len",))
def pallas_sequential_preLN__memory_aug_recurrent_mem_tr__swiglu_ffn__prompt_kernel(
    A_x: jax.Array,
    A_mem0: jax.Array,
    A_Wq: jax.Array,
    A_Wk: jax.Array,
    A_Wv: jax.Array,
    A_Wo: jax.Array,
    A_seg_len: int,
    B_x: jax.Array,
    B_w_gate: jax.Array,
    B_w_up: jax.Array,
    B_w_down: jax.Array,
):
    del B_x
    B, S, Dm = A_x.shape
    _, H, Dh = A_Wq.shape
    M = A_mem0.shape[1]
    F = B_w_gate.shape[1]
    seg = A_seg_len
    NP, PW = H // 2, 2 * Dh
    n_seg = S // seg
    assert B == 1 and PW == 3 * LANES and M == 8 and seg % 16 == 0 and S % seg == 0
    assert n_seg * M // LANES >= 3 and n_seg * M % LANES == 0
    assert (n_seg - 1) % UNROLL == 0 and NF <= LAG_WO
    assert H * Dh % (NP - RING) == 0 and F % ((NP - RING) * LANES) == 0

    def wt(w):
        return jnp.transpose(w, (1, 2, 0)).reshape(H * Dh, Dm)

    hbm = pl.BlockSpec(memory_space=pl.ANY)
    out = pl.pallas_call(
        functools.partial(_body, S=S, Dm=Dm, H=H, Dh=Dh, M=M, seg=seg, F=F),
        out_shape=jax.ShapeDtypeStruct((S, Dm), A_x.dtype),
        in_specs=[hbm, pl.BlockSpec(memory_space=pltpu.VMEM)] + [hbm] * 7,
        out_specs=hbm,
        scratch_shapes=[
            pltpu.VMEM((n_seg, seg, Dm), BF16),
            pltpu.VMEM((n_seg, M, Dm), BF16),
            pltpu.VMEM((n_seg * M, Dm), BF16),
            pltpu.VMEM((NP, n_seg * M, 3 * PW), F32),
            pltpu.VMEM((seg, Dm), F32),
            pltpu.VMEM((S, Dm), BF16),
            pltpu.VMEM((RING, 3, PW, Dm), BF16),
            pltpu.VMEM((NP, Dm // 2, 3 * PW), U32),
            pltpu.VMEM((H * Dh, Dm), BF16),
            pltpu.VMEM((Dm, F), BF16),
            pltpu.VMEM((Dm, F), BF16),
            pltpu.VMEM((F, Dm), BF16),
            pltpu.SemaphoreType.DMA((RING * 3,)),
            pltpu.SemaphoreType.DMA((1,)),
            pltpu.SemaphoreType.DMA((3,)),
            pltpu.SemaphoreType.DMA((3,)),
        ],
        compiler_params=pltpu.CompilerParams(
            vmem_limit_bytes=110 << 20,
            disable_bounds_checks=True,
            flags={"XLA_TPU_EVENLY_DISTRIBUTE_CRITICAL_NODES": True},
        ),
    )(A_x.reshape(n_seg, seg, Dm), A_mem0.reshape(M, Dm), wt(A_Wq), wt(A_Wk), wt(A_Wv),
      A_Wo.reshape(H * Dh, Dm), B_w_gate, B_w_up, B_w_down)
    return out.reshape(B, S, Dm)
```

```python
import functools

import jax
import jax.numpy as jnp
from jax import lax
import jax.experimental.pallas as pl
import jax.experimental.pallas.tpu as pltpu

F32 = jnp.float32
BF16 = jnp.bfloat16
U32 = jnp.uint32

LANES = 128
RING = 4
UNROLL = 3
NF = 4
LAG_QK, LAG_PV, LAG_WO = 1, 3, 4


def _mm(a, b):
    return lax.dot_general(a, b, (((1,), (0,)), ((), ())), preferred_element_type=F32)


def _mm_nt(a, b):
    return lax.dot_general(a, b, (((1,), (1,)), ((), ())), preferred_element_type=F32)


def _ln(x):
    m = jnp.mean(x, axis=-1, keepdims=True)
    d = x - m
    v = jnp.mean(d * d, axis=-1, keepdims=True)
    return d * lax.rsqrt(v + 1e-5)


def _body(x_hbm, mem0_hbm, wq_hbm, wk_hbm, wv_hbm, wo_hbm, wg_hbm, wu_hbm, wd_hbm,
          out_hbm,
          mem_v, x_v, xq_v, xp_v, pre, h_v, out_v, stg, wqkv, wo, wg, wu, wd,
          sem_w, sem_o, sem_f, sem_m,
          *, S, Dm, H, Dh, M, seg, F):
    NP = H // 2
    PW = 2 * Dh
    L = M + seg
    n_seg = S // seg
    scale = Dh ** (-0.5)
    PR = M
    NC = n_seg * PR // LANES
    N1 = NP - RING
    OB = H * Dh // N1
    FB = F // N1
    FC = F // NF

    def wcopies(j):
        slot = j % RING
        return [pltpu.make_async_copy(src.at[pl.ds(j * PW, PW), :], stg.at[slot, i],
                                      sem_w.at[slot * 3 + i])
                for i, src in enumerate((wq_hbm, wk_hbm, wv_hbm))]

    def side_copies(j):
        ro = pl.ds(pl.multiple_of(j * OB, OB), OB)
        rf = pl.ds(pl.multiple_of(j * FB, FB), FB)
        return [pltpu.make_async_copy(wo_hbm.at[ro, :], wo.at[ro, :], sem_o.at[0]),
                pltpu.make_async_copy(wd_hbm.at[rf, :], wd.at[rf, :], sem_f.at[0]),
                pltpu.make_async_copy(wg_hbm.at[:, rf], wg.at[:, rf], sem_f.at[1]),
                pltpu.make_async_copy(wu_hbm.at[:, rf], wu.at[:, rf], sem_f.at[2])]

    OR = UNROLL * seg

    def ocopy(i):
        r = pl.ds(pl.multiple_of(i * OR, OR), OR)
        return pltpu.make_async_copy(out_v.at[r, :], out_hbm.at[r, :], sem_m.at[1])

    def ln_pre(c):
        n = LANES // PR
        xs = jnp.concatenate([xq_v[c * n + t].astype(F32) for t in range(n)], axis=0)
        xp_v[c * LANES:(c + 1) * LANES, :] = _ln(xs).astype(BF16)

    def transpose_w(j, i):
        for t in range(PW // LANES):
            blk = stg[j % RING, i, t * LANES:(t + 1) * LANES, :]
            c0 = i * PW + t * LANES
            wqkv[j, :, c0:c0 + LANES] = pltpu.bitcast(blk.astype(F32).T.astype(BF16), U32)

    def transpose_pair(j):
        for i in range(3):
            transpose_w(j, i)

    def project_pre(j, c0=0, c1=3 * PW, chunks=range(NC)):
        w = pltpu.bitcast(wqkv[j, :, c0:c1], BF16)
        for c in chunks:
            rows = slice(c * LANES, (c + 1) * LANES)
            pre[j, rows, c0:c1] = _mm(xp_v[rows, :], w)

    cp_p = pltpu.make_async_copy(x_hbm.at[:, pl.ds(0, PR), :], xq_v, sem_m.at[2])
    cp_x = pltpu.make_async_copy(x_hbm, x_v, sem_m.at[0])
    cp_m = pltpu.make_async_copy(mem0_hbm, mem_v, sem_m.at[3])
    w0 = wcopies(0)
    cp_p.start()
    w0[0].start()
    cp_p.wait()
    w0[1].start()
    w0[2].start()
    w0[0].wait()
    for cp in wcopies(1):
        cp.start()
    transpose_w(0, 0)
    for c in range(NC):
        ln_pre(c)
    project_pre(0, 0, PW)
    w0[1].wait()
    w0[2].wait()
    for j in range(2, RING):
        for cp in wcopies(j):
            cp.start()
    transpose_w(0, 1)
    transpose_w(0, 2)
    project_pre(0, PW, 2 * PW)
    for cp in wcopies(1):
        cp.wait()
    for cp in wcopies(RING) + side_copies(0) + [cp_x, cp_m]:
        cp.start()
    transpose_pair(1)
    project_pre(0, 2 * PW, 3 * PW)

    def pro_body(i, carry):
        j = i + 1
        for cp in wcopies(j + 1):
            cp.wait()

        @pl.when(j < N1)
        def _():
            for cp in wcopies(j + RING) + side_copies(j):
                cp.start()

        transpose_pair(j + 1)
        project_pre(j)
        return carry

    lax.fori_loop(0, NP - 2, pro_body, 0)
    pltpu.make_async_copy(wo, wo, sem_o.at[0]).wait()
    pltpu.make_async_copy(wd, wd, sem_f.at[0]).wait()
    cp_x.wait()
    cp_m.wait()
    pltpu.make_async_copy(wg, wg, sem_f.at[1]).wait()
    pltpu.make_async_copy(wu, wu, sem_f.at[2]).wait()

    row = lax.broadcasted_iota(jnp.int32, (2 * L, 2 * L), 0)
    col = lax.broadcasted_iota(jnp.int32, (2 * L, 2 * L), 1)
    same_head = (row >= L) == (col >= L)
    r_in = jnp.where(row >= L, row - L, row)
    c_in = jnp.where(col >= L, col - L, col)
    valid = same_head & ((r_in < M) | (r_in >= c_in))
    fill = jnp.where(same_head, -1e9, -jnp.inf).astype(F32)
    lo = lax.broadcasted_iota(jnp.int32, (L, LANES), 1) < (Dh - LANES)

    def split_shared(t):
        return jnp.concatenate([jnp.where(lo, t, 0.0), jnp.where(lo, 0.0, t)], axis=0).astype(BF16)

    def ffn_gate_up(hn, c):
        g = _mm(hn, wg[:, c * FC:(c + 1) * FC])
        u = _mm(hn, wu[:, c * FC:(c + 1) * FC])
        return (g * (1.0 / (1.0 + jnp.exp(-g))) * u).astype(BF16)

    def ffn_down(h, acts):
        for c in range(NF):
            h = h + _mm(acts[c], wd[c * FC:(c + 1) * FC, :])
        return h

    def step_input(mem, s):
        return jnp.concatenate([mem, _ln(x_v[s, PR:, :].astype(F32))], axis=0).astype(BF16)

    def step(s, hin, first=False):
        rq = 0 if first else pl.multiple_of(s * PR, PR)
        if not first:
            h_prev = h_v[...]
            hn = _ln(h_prev).astype(BF16)
        st = {}
        acts = []

        def project(j):
            y = _mm(hin, pltpu.bitcast(wqkv[j], BF16))
            st["qkv", j] = jnp.concatenate([y[:M], pre[j, pl.ds(rq, PR), :], y[M:]], axis=0)

        def scores(j):
            y = st.pop(("qkv", j))
            t = [y[:, i * LANES:(i + 1) * LANES] for i in range(9)]
            qm = jnp.concatenate([t[0], t[2]], axis=0)
            km = jnp.concatenate([t[3], t[5]], axis=0).astype(BF16)
            kt = split_shared(t[4])
            st["vm", j] = jnp.concatenate([t[6], t[8]], axis=0).astype(BF16)
            st["vt", j] = split_shared(t[7])
            sm = _mm_nt(qm, km)
            stl = _mm_nt(t[1], kt)
            sc = (sm + jnp.concatenate([stl, stl], axis=0)) * scale
            sc = jnp.where(valid, sc, fill)
            e = jnp.exp(sc - jnp.max(sc, axis=-1, keepdims=True))
            st["p", j] = e / jnp.sum(e, axis=-1, keepdims=True)

        def mix(j):
            p = st.pop(("p", j))
            om = _mm(p, st.pop(("vm", j)))
            ot = _mm(p[:L] + p[L:], st.pop(("vt", j)))
            st["o", j] = jnp.concatenate([om[:L], ot, om[L:]], axis=1)

        def out_proj(j):
            y = _mm(st.pop(("o", j)), wo[j * PW:(j + 1) * PW, :])
            st["acc"] = y if j == 0 else st["acc"] + y

        for t in range(NP + LAG_WO):
            if t < NP:
                project(t)
            elif t - NP < NF and not first:
                acts.append(ffn_gate_up(hn, t - NP))
            if first:
                c = {NP - 2: 0, NP + 1: 1, NP + 2: 2}.get(t)
                if c is not None:
                    project_pre(NP - 1, chunks=(c,))
            if 0 <= t - LAG_WO < NP:
                out_proj(t - LAG_WO)
            if 0 <= t - LAG_PV < NP:
                mix(t - LAG_PV)
            if 0 <= t - LAG_QK < NP:
                scores(t - LAG_QK)
        if first:
            project_pre(NP - 1, chunks=range(3, NC))
        else:
            rp = pl.multiple_of((s - 1) * seg, seg)
            out_v[pl.ds(rp, seg), :] = ffn_down(h_prev, acts).astype(BF16)
        acc = st["acc"]
        h_v[...] = x_v[s].astype(F32) + acc[M:]
        return step_input(acc[:M], 1 if first else jnp.minimum(s + 1, n_seg - 1))

    def steps(i, hin):
        @pl.when(i >= 1)
        def _():
            ocopy(i - 1).start()

        for u in range(UNROLL):
            hin = step(1 + i * UNROLL + u, hin)
        return hin

    n_it = (n_seg - 1) // UNROLL
    hin = step(0, step_input(mem_v[...].astype(F32), 0), first=True)
    lax.fori_loop(0, n_it, steps, hin)

    ocopy(n_it - 1).start()
    h_prev = h_v[...]
    hn = _ln(h_prev).astype(BF16)
    acts = [ffn_gate_up(hn, c) for c in range(NF)]
    last = pl.ds(S - seg, seg)
    out_v[last, :] = ffn_down(h_prev, acts).astype(BF16)
    pltpu.make_async_copy(out_v.at[last, :], out_hbm.at[last, :], sem_m.at[1]).start()
    pltpu.make_async_copy(out_v, out_hbm, sem_m.at[1]).wait()


@functools.partial(jax.jit, static_argnames=("A_seg_len",))
def pallas_sequential_preLN__memory_aug_recurrent_mem_tr__swiglu_ffn__prompt_kernel(
    A_x: jax.Array,
    A_mem0: jax.Array,
    A_Wq: jax.Array,
    A_Wk: jax.Array,
    A_Wv: jax.Array,
    A_Wo: jax.Array,
    A_seg_len: int,
    B_x: jax.Array,
    B_w_gate: jax.Array,
    B_w_up: jax.Array,
    B_w_down: jax.Array,
):
    del B_x
    B, S, Dm = A_x.shape
    _, H, Dh = A_Wq.shape
    M = A_mem0.shape[1]
    F = B_w_gate.shape[1]
    seg = A_seg_len
    NP, PW = H // 2, 2 * Dh
    n_seg = S // seg
    assert B == 1 and PW == 3 * LANES and M == 8 and seg % 16 == 0 and S % seg == 0
    assert n_seg * M // LANES >= 3 and n_seg * M % LANES == 0
    assert (n_seg - 1) % UNROLL == 0 and NF <= LAG_WO
    assert H * Dh % (NP - RING) == 0 and F % ((NP - RING) * LANES) == 0

    def wt(w):
        return jnp.transpose(w, (1, 2, 0)).reshape(H * Dh, Dm)

    hbm = pl.BlockSpec(memory_space=pl.ANY)
    out = pl.pallas_call(
        functools.partial(_body, S=S, Dm=Dm, H=H, Dh=Dh, M=M, seg=seg, F=F),
        out_shape=jax.ShapeDtypeStruct((S, Dm), A_x.dtype),
        in_specs=[hbm] * 9,
        out_specs=hbm,
        scratch_shapes=[
            pltpu.VMEM((M, Dm), BF16),
            pltpu.VMEM((n_seg, seg, Dm), BF16),
            pltpu.VMEM((n_seg, M, Dm), BF16),
            pltpu.VMEM((n_seg * M, Dm), BF16),
            pltpu.VMEM((NP, n_seg * M, 3 * PW), F32),
            pltpu.VMEM((seg, Dm), F32),
            pltpu.VMEM((S, Dm), BF16),
            pltpu.VMEM((RING, 3, PW, Dm), BF16),
            pltpu.VMEM((NP, Dm // 2, 3 * PW), U32),
            pltpu.VMEM((H * Dh, Dm), BF16),
            pltpu.VMEM((Dm, F), BF16),
            pltpu.VMEM((Dm, F), BF16),
            pltpu.VMEM((F, Dm), BF16),
            pltpu.SemaphoreType.DMA((RING * 3,)),
            pltpu.SemaphoreType.DMA((1,)),
            pltpu.SemaphoreType.DMA((3,)),
            pltpu.SemaphoreType.DMA((4,)),
        ],
        compiler_params=pltpu.CompilerParams(
            vmem_limit_bytes=110 << 20,
            disable_bounds_checks=True,
            flags={"XLA_TPU_EVENLY_DISTRIBUTE_CRITICAL_NODES": True},
        ),
    )(A_x.reshape(n_seg, seg, Dm), A_mem0.reshape(M, Dm), wt(A_Wq), wt(A_Wk), wt(A_Wv),
      A_Wo.reshape(H * Dh, Dm), B_w_gate, B_w_up, B_w_down)
    return out.reshape(B, S, Dm)
```
